```python
import os as _os
_os.environ.setdefault("JAX_PLATFORMS", "cpu")
import jax
import jax.numpy as jnp

def _softmax(x, axis=-1):
    return jax.nn.softmax(x, axis=axis)
def _gelu(x):
    return jax.nn.gelu(x, approximate=True)
def _silu(x):
    return jax.nn.silu(x)
def _sigmoid(x):
    return jax.nn.sigmoid(x)
def _layernorm(x, axis=-1, eps=1e-5):
    m = jnp.mean(x, axis=axis, keepdims=True)
    v = jnp.var(x, axis=axis, keepdims=True)
    return (x - m) / jnp.sqrt(v + eps)
def _scatter_add(tgt, idx, src, axis=0):
    return tgt.at[idx].add(src)
def _segment_sum(src, seg, n):
    return jax.ops.segment_sum(src, seg, n)
class _Rng:
    def __init__(self, key):
        self._k = key
    def _next(self):
        self._k, sub = jax.random.split(self._k)
        return sub
    def normal(self, shape):
        return jax.random.normal(self._next(), shape, dtype=jnp.bfloat16)
    def randint(self, lo, hi, shape):
        return jax.random.randint(self._next(), shape, lo, hi, dtype=jnp.int32)
    def uniform(self, shape, lo=0.0, hi=1.0):
        return jax.random.uniform(self._next(), shape, jnp.bfloat16, lo, hi)
    def permutation(self, n):
        return jax.random.permutation(self._next(), n)


kernel_name = 'standalone__mha_softmax__near_ridge'

def setup_inputs():
    _rng = _Rng(jax.random.key(int.from_bytes(__import__("os").urandom(4), "little")))
    _w = (lambda a: (lambda t: t.astype(jnp.bfloat16) if jnp.issubdtype(t.dtype, jnp.floating) else t)(jnp.asarray(a)))
    B, H, Sq, Sk, D = 8, 16, 192, 1024, 256
    return {
        "q": _w((lambda *s: _rng.normal(s) * 0.4)(B, H, Sq, D)),
        "k": _w((lambda *s: _rng.normal(s) * 0.4)(B, H, Sk, D)),
        "v": _w((lambda *s: _rng.normal(s) * 0.05)(B, H, Sk, D)),
    }

def reference(q, k, v):
    scale = q.shape[-1] ** -0.5
    scores = jnp.einsum("bhqd,bhkd->bhqk", q, k) * scale
    p = _softmax(scores, axis=-1)
    return jnp.einsum("bhqk,bhkd->bhqd", p, v)
```

```python
import math

import jax
import jax.numpy as jnp
import jax.experimental.pallas as pl
import jax.experimental.pallas.tpu as pltpu

_LOG2E = math.log2(math.e)
_NB = 3
_W_ROWS = 48
_W_STREAMS = 4


@jax.jit
def pallas_standalone__mha_softmax__near_ridge_kernel(
    q: jax.Array,
    k: jax.Array,
    v: jax.Array,
):
    B, H, Sq, D = q.shape
    Sk = k.shape[2]
    N = B * H
    c = (D ** -0.5) * _LOG2E

    def kernel(q_hbm, k_hbm, v_hbm, o_hbm, qbuf, kbuf, vbuf, obuf, sems, wsem):
        def loads(h, slot):
            return [
                (pltpu.make_async_copy(q_hbm.at[h], qbuf.at[slot], sems.at[0, slot]), 0),
                (pltpu.make_async_copy(k_hbm.at[h], kbuf.at[slot], sems.at[1, slot]), 0),
                (pltpu.make_async_copy(v_hbm.at[h], vbuf.at[slot], sems.at[2, slot]), 1),
            ]

        def attend(h, slot):
            s = jax.lax.dot_general(
                qbuf[slot], kbuf[slot], (((1,), (1,)), ((), ())),
                preferred_element_type=jnp.float32)
            m = jnp.max(s, axis=-1, keepdims=True)
            p = jnp.exp2((s - m) * c)
            l = jnp.sum(p, axis=-1, keepdims=True)
            o = jnp.dot(p.astype(vbuf.dtype), vbuf[slot],
                        preferred_element_type=jnp.float32)
            obuf[h] = (o * (1.0 / l)).astype(obuf.dtype)

        for j in range(_NB - 1):
            for cp, prio in loads(j, j):
                cp.start(priority=prio)

        def body(h, carry):
            @pl.when(h + _NB - 1 < N)
            def _():
                for cp, prio in loads(h + _NB - 1, (h + _NB - 1) % _NB):
                    cp.start(priority=prio)

            slot = h % _NB
            for cp, _ in loads(h, slot):
                cp.wait()
            attend(h, slot)
            return carry

        jax.lax.fori_loop(0, N - 1, body, 0)

        last = N - 1
        for cp, _ in loads(last, last % _NB):
            cp.wait()
        per = last // _W_STREAMS

        def write_back(j, carry):
            for r in range(Sq // _W_ROWS):
                rows = pl.ds(r * _W_ROWS, _W_ROWS)
                for s in range(_W_STREAMS):
                    h = s * per + j
                    pltpu.make_async_copy(
                        obuf.at[h, rows], o_hbm.at[h, rows], wsem.at[0]).start()
            return carry

        jax.lax.fori_loop(0, per, write_back, 0)
        for h in range(per * _W_STREAMS, last):
            pltpu.make_async_copy(obuf.at[h], o_hbm.at[h], wsem.at[0]).start()
        attend(last, last % _NB)
        pltpu.make_async_copy(obuf.at[last], o_hbm.at[last], wsem.at[0]).start()
        pltpu.make_async_copy(obuf, o_hbm, wsem.at[0]).wait()

    out = pl.pallas_call(
        kernel,
        in_specs=[pl.BlockSpec(memory_space=pl.ANY)] * 3,
        out_specs=pl.BlockSpec(memory_space=pl.ANY),
        out_shape=jax.ShapeDtypeStruct((N, Sq, D), q.dtype),
        scratch_shapes=[
            pltpu.VMEM((_NB, Sq, D), q.dtype),
            pltpu.VMEM((_NB, Sk, D), k.dtype),
            pltpu.VMEM((_NB, Sk, D), v.dtype),
            pltpu.VMEM((N, Sq, D), q.dtype),
            pltpu.SemaphoreType.DMA((3, _NB)),
            pltpu.SemaphoreType.DMA((1,)),
        ],
        compiler_params=pltpu.CompilerParams(vmem_limit_bytes=64 * 1024 * 1024),
    )(q.reshape(N, Sq, D), k.reshape(N, Sk, D), v.reshape(N, Sk, D))
    return out.reshape(B, H, Sq, D)
```

```python
import math

import jax
from jax import lax
import jax.experimental.pallas as pl
import jax.experimental.pallas.tpu as pltpu
import jax.numpy as jnp

_GROUP = 8
_RING = 3
_AHEAD = _GROUP + 1
_SEMS = _AHEAD - _GROUP + 1
_FAST = (4, 16)
_SLOW = (2, 64)
_KEY_BLOCK = 256
_FAST_V = (3, 3, 2)
_FAST_K = (2, 2, 2, 1, 1)
_OUT_REGION = 1024
_OUT_ROWS = 16
_OUT_STORE = 64
_SPIN = 9


@jax.jit
def pallas_standalone__mha_softmax__near_ridge_kernel(
    q: jax.Array,
    k: jax.Array,
    v: jax.Array,
):
    B, H, Sq, D = q.shape
    Sk = k.shape[2]
    N = B * H
    exp2_scale = (D ** -0.5) * math.log2(math.e)

    rounds = Sk // _KEY_BLOCK
    slice_rows = Sk // _GROUP
    slots = _RING * _GROUP
    n_fetching = N - _AHEAD
    n_regions = N * Sq // _OUT_REGION
    n_early = n_fetching * Sq // _OUT_REGION
    assert Sk % _KEY_BLOCK == 0 and N % _GROUP == 0 and N * Sq % _OUT_REGION == 0
    assert Sq % _OUT_STORE == 0 and 0 < n_early < n_regions

    per_round = {"v": _FAST_V, "k": _FAST_K}
    assert len(_FAST_V) == rounds - 1 and len(_FAST_K) == rounds + 1

    def pieces(first_row, end_row, heads, rows):
        return [(r, min(rows, end_row - r), h, heads)
                for r in range(first_row, end_row, rows) for h in range(0, _GROUP, heads)]

    fast, slow = {}, {"q": [(0, Sq, 0, 1)]}
    for t in "kv":
        fast_rows = sum(per_round[t]) * _FAST[0] // _GROUP * _FAST[1]
        fast[t] = pieces(0, fast_rows, *_FAST)
        slow[t] = pieces(fast_rows, slice_rows, *_SLOW)
        assert len(fast[t]) == sum(per_round[t]) and fast_rows <= slice_rows

    def kernel(q_hbm, k_hbm, v_hbm, o_hbm, q_buf, k_buf, v_buf, o_buf, in_sems, out_sem):
        refs = {"q": (q_hbm, q_buf, 0), "k": (k_hbm, k_buf, 1), "v": (v_hbm, v_buf, 2)}

        def copy(t, j, row0, rows, head0, heads):
            src, dst, s = refs[t]
            sem = in_sems.at[s, lax.rem(j, _SEMS)]
            if t == "q":
                return pltpu.make_async_copy(src.at[j], dst.at[lax.rem(j, slots)], sem)
            g = lax.div(j, _GROUP)
            band = pl.ds(pl.multiple_of(lax.rem(j, _GROUP) * slice_rows + row0, 16), rows)
            return pltpu.make_async_copy(
                src.at[pl.ds(g * _GROUP + head0, heads), band],
                dst.at[pl.ds(lax.rem(g, _RING) * _GROUP + head0, heads), band],
                sem)

        def start(t, j, piece, priority):
            copy(t, j, *piece).start(priority=priority)

        def wait_slice(j):
            for t in "qkv":
                copy(t, j, 0, slice_rows, 0, _GROUP).wait()

        def attend(h, fetch):
            slot = lax.rem(h, slots)

            def issue(t, i, result):
                if not fetch:
                    return
                buf = refs[t][1]
                first, count = sum(per_round[t][:i]), per_round[t][i]
                for x in range(first, first + count):
                    row = (x - first) * Sq // count // 16 * 16
                    buf[slots, 0:16, 0:128] = result[row:row + 16, 0:128].astype(buf.dtype)
                    start(t, h + _AHEAD, fast[t][x], 0)
                    lo = len(slow[t]) * x // len(fast[t])
                    hi = len(slow[t]) * (x + 1) // len(fast[t])
                    for piece in slow[t][lo:hi]:
                        start(t, h + _AHEAD, piece, 1)

            if fetch:
                start("q", h + _AHEAD, slow["q"][0], 1)

            qh = q_buf[slot]
            s_blocks = [
                lax.dot_general(
                    qh, k_buf[slot, pl.ds(r * _KEY_BLOCK, _KEY_BLOCK)],
                    (((1,), (1,)), ((), ())), preferred_element_type=jnp.float32)
                for r in range(rounds)
            ]
            for r in range(rounds - 1):
                issue("v", r, s_blocks[r])

            s = jnp.concatenate(s_blocks, axis=1)
            m = jnp.max(s, axis=-1, keepdims=True)
            p = jnp.exp2((s - m) * exp2_scale)
            l = jnp.sum(p, axis=-1, keepdims=True)
            p = p.astype(v_buf.dtype)
            issue("k", 0, s_blocks[-1])

            o = None
            for r in range(rounds):
                d = jnp.dot(
                    p[:, r * _KEY_BLOCK:(r + 1) * _KEY_BLOCK],
                    v_buf[slot, pl.ds(r * _KEY_BLOCK, _KEY_BLOCK)],
                    preferred_element_type=jnp.float32)
                o = d if o is None else o + d
                issue("k", r + 1, o)

            o = (o * (1.0 / l)).astype(o_buf.dtype)
            for i in range(Sq // _OUT_STORE):
                u = h * (Sq // _OUT_STORE) + i
                row = pl.multiple_of(
                    lax.rem(u, _OUT_REGION // _OUT_STORE) * _OUT_STORE, _OUT_STORE)
                o_buf[lax.div(u, _OUT_REGION // _OUT_STORE), pl.ds(row, _OUT_STORE)] = (
                    o[i * _OUT_STORE:(i + 1) * _OUT_STORE])

        k_buf[slots, 0:16, 0:128] = jnp.zeros((16, 128), k_buf.dtype)

        def start_up(j, carry):
            @pl.when(j >= _SEMS)
            def _():
                wait_slice(jnp.maximum(j - _SEMS, 0))

            for t in "qvk":
                for piece in slow[t]:
                    start(t, j, piece, 1)
            for t in "vk":
                for piece in fast[t]:
                    start(t, j, piece, 0)
                    idle = lax.fori_loop(
                        0, _SPIN, lambda _, y: y * 0.5 + 1.0,
                        k_buf[slots, 0:16, 0:128].astype(jnp.float32))
                    k_buf[slots, 0:16, 0:128] = idle.astype(k_buf.dtype)
            return carry

        lax.fori_loop(0, _AHEAD, start_up, 0)

        def steady(h, carry):
            wait_slice(h + _GROUP - 1)
            attend(h, fetch=True)
            return carry

        lax.fori_loop(0, n_fetching, steady, 0)

        def write_back(first, count):
            def body(i, carry):
                where = (pl.ds(first, count),
                         pl.ds(pl.multiple_of(i * _OUT_ROWS, _OUT_ROWS), _OUT_ROWS))
                pltpu.make_async_copy(
                    o_buf.at[where], o_hbm.at[where], out_sem.at[0]).start(priority=1)
                return carry

            lax.fori_loop(0, _OUT_REGION // _OUT_ROWS, body, 0)

        write_back(0, n_early)

        def drain(h, carry):
            @pl.when(h + _GROUP - 1 < N)
            def _():
                wait_slice(jnp.minimum(h + _GROUP - 1, N - 1))

            attend(h, fetch=False)
            return carry

        lax.fori_loop(n_fetching, N, drain, 0)

        write_back(n_early, n_regions - n_early)
        pltpu.make_async_copy(o_buf, o_hbm, out_sem.at[0]).wait()

    out = pl.pallas_call(
        kernel,
        in_specs=[pl.BlockSpec(memory_space=pl.ANY)] * 3,
        out_specs=pl.BlockSpec(memory_space=pl.ANY),
        out_shape=jax.ShapeDtypeStruct((n_regions, _OUT_REGION, D), q.dtype),
        scratch_shapes=[
            pltpu.VMEM((slots, Sq, D), q.dtype),
            pltpu.VMEM((slots + 1, Sk, D), k.dtype),
            pltpu.VMEM((slots + 1, Sk, D), v.dtype),
            pltpu.VMEM((n_regions, _OUT_REGION, D), q.dtype),
            pltpu.SemaphoreType.DMA((3, _SEMS)),
            pltpu.SemaphoreType.DMA((1,)),
        ],
        compiler_params=pltpu.CompilerParams(vmem_limit_bytes=64 * 1024 * 1024),
    )(q.reshape(N, Sq, D), k.reshape(N, Sk, D), v.reshape(N, Sk, D))
    return out.reshape(B, H, Sq, D)
```
